```python
import jax
import jax.numpy as jnp

def _softmax(x, axis=-1):
    return jax.nn.softmax(x, axis=axis)
def _gelu(x):
    return jax.nn.gelu(x, approximate=True)
def _silu(x):
    return jax.nn.silu(x)
def _sigmoid(x):
    return jax.nn.sigmoid(x)
def _layernorm(x, axis=-1, eps=1e-5):
    m = jnp.mean(x, axis=axis, keepdims=True)
    v = jnp.var(x, axis=axis, keepdims=True)
    return (x - m) / jnp.sqrt(v + eps)
def _scatter_add(tgt, idx, src, axis=0):
    return tgt.at[idx].add(src)
def _segment_sum(src, seg, n):
    return jax.ops.segment_sum(src, seg, n)
class _Rng:
    def __init__(self, key):
        self._k = key
    def _next(self):
        self._k, sub = jax.random.split(self._k)
        return sub
    def normal(self, shape):
        return jax.random.normal(self._next(), shape, dtype=jnp.bfloat16)
    def randint(self, lo, hi, shape):
        return jax.random.randint(self._next(), shape, lo, hi, dtype=jnp.int32)
    def uniform(self, shape, lo=0.0, hi=1.0):
        return jax.random.uniform(self._next(), shape, jnp.bfloat16, lo, hi)
    def permutation(self, n):
        return jax.random.permutation(self._next(), n)


kernel_name = 'gated_mix__sliding_block_cached__glu_gated_swiglu__decode'

def setup_inputs():
    _rng = _Rng(jax.random.key(int.from_bytes(__import__("os").urandom(4), "little")))
    _w = (lambda a: (lambda t: t.astype(jnp.bfloat16) if jnp.issubdtype(t.dtype, jnp.floating) else t)(jnp.asarray(a)))
    def _A_setup():
        B, Sq, D = 1, 1, 640
        Hq, Hkv, Sk, Dh = 32, 32, 32768, 192
        assert Hq % Hkv == 0, (Hq, Hkv)
        return {
            "x": _w((lambda *s: _rng.normal(s) * 0.05)(B, Sq, D)),
            "k_cache": _w((lambda *s: _rng.normal(s) * 0.05)(B, Hkv, Sk, Dh)),
            "v_cache": _w((lambda *s: _rng.normal(s) * 0.05)(B, Hkv, Sk, Dh)),
            "wq": _w((lambda *s: _rng.normal(s) * 0.05)(D, Hq * Dh) * (D ** -0.5)),
            "wo": _w((lambda *s: _rng.normal(s) * 0.05)(Hq * Dh, D) * ((Hq * Dh) ** -0.5)),
        }
    _A_in = _A_setup()

    def _B_setup():
        B, S, D, F = 1, 1, 640, 1536
        return {
            "x": _w((lambda *s: _rng.normal(s) * 0.05)(B, S, D)),
            "w1": _w((lambda *s: _rng.normal(s) * 0.05)(D, F) * (2.0 / D) ** 0.5),
            "w3": _w((lambda *s: _rng.normal(s) * 0.05)(D, F) * (2.0 / D) ** 0.5),
            "w2": _w((lambda *s: _rng.normal(s) * 0.05)(F, D) * (2.0 / F) ** 0.5),
        }
    _B_in = _B_setup()

    return {
        "A_x": _A_in["x"],
        "A_k_cache": _A_in["k_cache"],
        "A_v_cache": _A_in["v_cache"],
        "A_wq": _A_in["wq"],
        "A_wo": _A_in["wo"],
        "B_x": _B_in["x"],
        "B_w1": _B_in["w1"],
        "B_w3": _B_in["w3"],
        "B_w2": _B_in["w2"],
        "gate_w": _w((lambda *s: _rng.normal(s) * 0.05)(640)),
    }

def reference(A_x, A_k_cache, A_v_cache, A_wq, A_wo, B_x, B_w1, B_w3, B_w2, gate_w):
    def _A_ref(x, k_cache, v_cache, wq, wo):
        B, Sq, D = x.shape
        Hq, Dh = 32, 192
        Hkv, Sk = k_cache.shape[1], k_cache.shape[2]
        W = min(4096, max(256, Sk // 4))
        rep = Hq // Hkv
        q = (lambda x, *d: x.transpose(*d))((x @ wq).reshape(B, Sq, Hq, Dh), 0, 2, 1, 3)
        k = jnp.repeat(k_cache[:, :, Sk - W:, :], rep, axis=1)
        v = jnp.repeat(v_cache[:, :, Sk - W:, :], rep, axis=1)
        scores = jnp.einsum("bhqd,bhkd->bhqk", q, k) * (Dh ** -0.5)
        p = _softmax(scores, axis=-1)
        o = jnp.einsum("bhqk,bhkd->bhqd", p, v)
        return (lambda x, *d: x.transpose(*d))(o, 0, 2, 1, 3).reshape(B, Sq, Hq * Dh) @ wo

    def _B_ref(x, w1, w3, w2):
        gate = jnp.einsum("bsd,df->bsf", x, w1)
        up = jnp.einsum("bsd,df->bsf", x, w3)
        h = _silu(gate) * up
        out = jnp.einsum("bsf,fd->bsd", h, w2)
        return out

    x = A_x
    g = _sigmoid((x * gate_w).sum(-1, keepdims=True))
    a = _A_ref(x, A_k_cache, A_v_cache, A_wq, A_wo)
    b = _B_ref(x, B_w1, B_w3, B_w2)
    return g * a + (1 - g) * b
```

```python
import jax
import jax.numpy as jnp
from jax import lax
import jax.experimental.pallas as pl
import jax.experimental.pallas.tpu as pltpu

_NT = (((1,), (1,)), ((), ()))


@jax.jit
def pallas_gated_mix__sliding_block_cached__glu_gated_swiglu__decode_kernel(
    A_x: jax.Array,
    A_k_cache: jax.Array,
    A_v_cache: jax.Array,
    A_wq: jax.Array,
    A_wo: jax.Array,
    B_x: jax.Array,
    B_w1: jax.Array,
    B_w3: jax.Array,
    B_w2: jax.Array,
    gate_w: jax.Array,
):
    del B_x
    B, Sq, D = A_x.shape
    _, H, SK, DH = A_k_cache.shape
    F = B_w1.shape[1]
    W = min(4096, max(256, SK // 4))
    nk = nv = 4
    scale = DH ** -0.5

    kT = jnp.swapaxes(A_k_cache, 2, 3).reshape(H * DH, SK)
    vT = jnp.swapaxes(A_v_cache, 2, 3).reshape(H * DH, SK)

    def kernel(x_ref, k_ref, v_ref, wq_ref, wo_ref, w1_ref, w3_ref, w2_ref, gw_ref, o_ref,
               kbuf, vbuf, wq_b, wo_b, w1_b, w3_b, w2_b, q_s, ksem, vsem, wsems):
        def kcopy(h):
            return pltpu.make_async_copy(k_ref.at[pl.ds(h * DH, DH), pl.ds(SK - W, W)], kbuf.at[h % nk], ksem.at[h % nk])

        def vcopy(h):
            return pltpu.make_async_copy(v_ref.at[pl.ds(h * DH, DH), pl.ds(SK - W, W)], vbuf.at[h % nv], vsem.at[h % nv])

        cq = pltpu.make_async_copy(wq_ref, wq_b, wsems.at[0])
        c1 = pltpu.make_async_copy(w1_ref, w1_b, wsems.at[1])
        c3 = pltpu.make_async_copy(w3_ref, w3_b, wsems.at[2])
        c2 = pltpu.make_async_copy(w2_ref, w2_b, wsems.at[3])
        co = pltpu.make_async_copy(wo_ref, wo_b, wsems.at[4])
        cq.start()
        kcopy(0).start()
        vcopy(0).start()
        co.start()
        for h in range(1, min(nk, nv)):
            kcopy(h).start()
            vcopy(h).start()
        x = x_ref[0]
        xb = jnp.broadcast_to(x, (8, D))
        cq.wait()
        q = jnp.dot(xb, wq_b[...], preferred_element_type=jnp.float32)
        q_s[...] = q.astype(jnp.bfloat16).astype(jnp.float32)
        acc = jnp.zeros((8, D), jnp.float32)
        for h in range(H):
            kcopy(h).wait()
            qh = q_s[:, h * DH:(h + 1) * DH].astype(jnp.bfloat16)
            s = jnp.dot(qh, kbuf[h % nk], preferred_element_type=jnp.float32) * scale
            if h + nk < H:
                kcopy(h + nk).start()
            m = jnp.max(s, axis=-1, keepdims=True)
            e = jnp.exp(s - m)
            l = jnp.sum(e, axis=-1, keepdims=True)
            p = (e / l).astype(jnp.bfloat16)
            vcopy(h).wait()
            o = lax.dot_general(p, vbuf[h % nv], _NT, preferred_element_type=jnp.float32)
            if h + nv < H:
                vcopy(h + nv).start()
            if h == 0:
                co.wait()
            if h == 8:
                c1.start()
                c3.start()
                c2.start()
            acc = acc + jnp.dot(o.astype(jnp.bfloat16), wo_b[h * DH:(h + 1) * DH, :], preferred_element_type=jnp.float32)
        c1.wait()
        c3.wait()
        c2.wait()
        g_ = jnp.dot(xb, w1_b[...], preferred_element_type=jnp.float32)
        u_ = jnp.dot(xb, w3_b[...], preferred_element_type=jnp.float32)
        hh = (g_ * jax.nn.sigmoid(g_) * u_).astype(jnp.bfloat16)
        b = jnp.dot(hh, w2_b[...], preferred_element_type=jnp.float32)
        gw = gw_ref[...].reshape(1, D).astype(jnp.float32)
        gl = jnp.sum(x.astype(jnp.float32) * gw, axis=-1, keepdims=True)
        g = jax.nn.sigmoid(gl)
        out = g * acc[0:1] + (1 - g) * b[0:1]
        o_ref[0] = out.astype(jnp.bfloat16)

    any_spec = pl.BlockSpec(memory_space=pl.ANY)
    vm = pl.BlockSpec(memory_space=pltpu.VMEM)
    return pl.pallas_call(
        kernel,
        out_shape=jax.ShapeDtypeStruct((B, Sq, D), A_x.dtype),
        in_specs=[vm] + [any_spec] * 7 + [vm],
        out_specs=vm,
        scratch_shapes=[
            pltpu.VMEM((nk, DH, W), jnp.bfloat16),
            pltpu.VMEM((nv, DH, W), jnp.bfloat16),
            pltpu.VMEM((D, H * DH), jnp.bfloat16),
            pltpu.VMEM((H * DH, D), jnp.bfloat16),
            pltpu.VMEM((D, F), jnp.bfloat16),
            pltpu.VMEM((D, F), jnp.bfloat16),
            pltpu.VMEM((F, D), jnp.bfloat16),
            pltpu.VMEM((8, H * DH), jnp.float32),
            pltpu.SemaphoreType.DMA((nk,)),
            pltpu.SemaphoreType.DMA((nv,)),
            pltpu.SemaphoreType.DMA((5,)),
        ],
        compiler_params=pltpu.CompilerParams(vmem_limit_bytes=64 * 1024 * 1024),
    )(A_x, kT, vT, A_wq, A_wo, B_w1, B_w3, B_w2, gate_w)
```

```python
import jax
import jax.numpy as jnp
from jax import lax
import jax.experimental.pallas as pl
import jax.experimental.pallas.tpu as pltpu

_NT = (((1,), (1,)), ((), ()))


@jax.jit
def pallas_gated_mix__sliding_block_cached__glu_gated_swiglu__decode_kernel(
    A_x: jax.Array,
    A_k_cache: jax.Array,
    A_v_cache: jax.Array,
    A_wq: jax.Array,
    A_wo: jax.Array,
    B_x: jax.Array,
    B_w1: jax.Array,
    B_w3: jax.Array,
    B_w2: jax.Array,
    gate_w: jax.Array,
):
    del B_x
    B, Sq, D = A_x.shape
    _, H, SK, DH = A_k_cache.shape
    F = B_w1.shape[1]
    W = min(4096, max(256, SK // 4))
    scale = DH ** -0.5
    ROWS, cols, wo_rows, wq_cols = 8, 2048, 24, 2048
    nrb = DH // ROWS
    ncb = W // cols
    per = nrb * ncb
    tot = 2 * per
    lag = tot
    rc = [(r, c) for c in range(ncb) for r in range(nrb)]

    kT = jnp.swapaxes(A_k_cache, 2, 3).reshape(H * DH, SK)
    vT = jnp.swapaxes(A_v_cache, 2, 3).reshape(H * DH, SK)

    def kernel(x_ref, k_ref, v_ref, wq_ref, wo_ref, w1_ref, w3_ref, w2_ref, gw_ref, o_ref,
               kvbuf, wq_b, wo_b, w1_b, w3_b, w2_b, x_b, gw_b, q_s, kvsem, wsem):
        def kvcp(h, slot, j):
            m = j // per
            r, c = rc[j % per]
            src = k_ref if m == 0 else v_ref
            row = h * DH + r * ROWS
            if not isinstance(row, int):
                row = pl.multiple_of(row, 8)
            return pltpu.make_async_copy(
                src.at[pl.ds(row, ROWS), pl.ds(SK - W + c * cols, cols)],
                kvbuf.at[slot * 2 + m, pl.ds(r * ROWS, ROWS), pl.ds(c * cols, cols)],
                kvsem.at[slot * 2 + m])

        def rows_chunks(src, dst, rows, sem, cw=None):
            R = src.shape[0]
            out = []
            if cw is None:
                for r in range(R // rows):
                    out.append((src.at[pl.ds(r * rows, rows), :], dst.at[pl.ds(r * rows, rows), :], sem))
            else:
                for c in range(src.shape[1] // cw):
                    for r in range(R // rows):
                        out.append((src.at[pl.ds(r * rows, rows), pl.ds(c * cw, cw)],
                                    dst.at[pl.ds(r * rows, rows), pl.ds(c * cw, cw)], sem))
            return out

        def stride_order(lst, S):
            return [lst[j] for off in range(S) for j in range(off, len(lst), S)]

        def merge(*ls):
            pos = []
            for a, l in enumerate(ls):
                for i, e in enumerate(l):
                    pos.append(((i + 0.5) / len(l), a, e))
            pos.sort(key=lambda t: (t[0], t[1]))
            return [e for _, _, e in pos]

        s_w13, s_w2, s_wo, s_wq, s_x = (wsem.at[i] for i in range(5))
        c_w1 = rows_chunks(w1_ref, w1_b, 8, s_w13)
        c_w3 = rows_chunks(w3_ref, w3_b, 8, s_w13)
        c_w2 = rows_chunks(w2_ref, w2_b, wo_rows, s_w2)
        c_wo = stride_order(rows_chunks(wo_ref, wo_b, wo_rows, s_wo), 16)
        c_wq = stride_order(rows_chunks(wq_ref, wq_b, 8, s_wq, cw=wq_cols), 4)
        pro = merge(c_wq, c_w1, c_w3, c_w2) + c_wo
        P = len(pro)

        def mk(i):
            if i < P:
                s, d, sem = pro[i]
                return pltpu.make_async_copy(s, d, sem)
            i -= P
            h = i // tot
            return kvcp(h, h % 2, i % tot)

        cx = pltpu.make_async_copy(x_ref, x_b, s_x)
        cg = pltpu.make_async_copy(gw_ref, gw_b, s_x)
        for i in range(lag):
            mk(i).start(priority=i % 2)
            if i == 1:
                cx.start()
                cg.start()
        for i in range(P):
            mk(i).wait()
            mk(i + lag).start(priority=(i + lag) % 2)
        cx.wait()
        cg.wait()
        x = x_b[0]
        xb = jnp.broadcast_to(x, (8, D))
        q = jnp.dot(xb, wq_b[...], preferred_element_type=jnp.float32)
        qb = q.astype(jnp.bfloat16)
        for h in range(H):
            q_s[h] = qb[:, h * DH:(h + 1) * DH]
        g_ = jnp.dot(xb, w1_b[...], preferred_element_type=jnp.float32)
        u_ = jnp.dot(xb, w3_b[...], preferred_element_type=jnp.float32)
        hh = (g_ * jax.nn.sigmoid(g_) * u_).astype(jnp.bfloat16)
        b = jnp.dot(hh, w2_b[...], preferred_element_type=jnp.float32)
        gwv = gw_b[...].reshape(1, D).astype(jnp.float32)
        gl = jnp.sum(x.astype(jnp.float32) * gwv, axis=-1, keepdims=True)
        g = jax.nn.sigmoid(gl)

        def head(h, acc, last):
            slot = h % 2
            nslot = 1 - slot
            par = P % 2
            for j in range(per):
                kvcp(h, slot, j).wait()
                if not last:
                    kvcp(h + 1, nslot, j).start(priority=(j + par) % 2)
            s = jnp.dot(q_s[h], kvbuf[slot * 2], preferred_element_type=jnp.float32) * scale
            m = jnp.max(s, axis=-1, keepdims=True)
            e = jnp.exp(s - m)
            l = jnp.sum(e, axis=-1, keepdims=True)
            p = (e / l).astype(jnp.bfloat16)
            for j in range(per, tot):
                kvcp(h, slot, j).wait()
                if not last:
                    kvcp(h + 1, nslot, j).start(priority=(j + par) % 2)
            o = lax.dot_general(p, kvbuf[slot * 2 + 1], _NT, preferred_element_type=jnp.float32)
            row = h * DH
            if not isinstance(row, int):
                row = pl.multiple_of(row, 64)
            return acc + jnp.dot(o.astype(jnp.bfloat16), wo_b[pl.ds(row, DH), :],
                                 preferred_element_type=jnp.float32)

        acc = lax.fori_loop(0, H - 1, lambda h, a: head(h, a, False), jnp.zeros((8, D), jnp.float32))
        acc = head(H - 1, acc, True)
        out = g * acc[0:1] + (1 - g) * b[0:1]
        o_ref[0] = out.astype(o_ref.dtype)

    any_spec = pl.BlockSpec(memory_space=pl.ANY)
    return pl.pallas_call(
        kernel,
        out_shape=jax.ShapeDtypeStruct((B, Sq, D), A_x.dtype),
        in_specs=[any_spec] * 9,
        out_specs=pl.BlockSpec(memory_space=pltpu.VMEM),
        scratch_shapes=[
            pltpu.VMEM((4, DH, W), jnp.bfloat16),
            pltpu.VMEM((D, H * DH), jnp.bfloat16),
            pltpu.VMEM((H * DH, D), jnp.bfloat16),
            pltpu.VMEM((D, F), jnp.bfloat16),
            pltpu.VMEM((D, F), jnp.bfloat16),
            pltpu.VMEM((F, D), jnp.bfloat16),
            pltpu.VMEM((1, 1, D), jnp.bfloat16),
            pltpu.VMEM((D,), jnp.bfloat16),
            pltpu.VMEM((H, 8, DH), jnp.bfloat16),
            pltpu.SemaphoreType.DMA((4,)),
            pltpu.SemaphoreType.DMA((5,)),
        ],
        compiler_params=pltpu.CompilerParams(vmem_limit_bytes=48 * 1024 * 1024),
    )(A_x, kT, vT, A_wq, A_wo, B_w1, B_w3, B_w2, gate_w)
```

```python
import jax
import jax.numpy as jnp
from jax import lax
import jax.experimental.pallas as pl
import jax.experimental.pallas.tpu as pltpu

_NT = (((1,), (1,)), ((), ()))
_F32 = jnp.float32
_BF16 = jnp.bfloat16

_LAG = 72
_NSEM = 4
_COLS = 2048
_STRIDE = 16
_TAIL = (6, 3, 2, 1)
_TAIL_P1_FROM = 2


def _aligned_pieces(R, C, r0=0, r1=None, ntiles=16):
    r1 = R if r1 is None else r1
    tpr = C // 128
    ta, tb = (r0 // 8) * tpr, (r1 // 8) * tpr
    bounds = sorted(set([ta, tb] + [t for t in range(0, (R // 8) * tpr + 1, ntiles) if ta < t < tb]))
    pieces = []
    for t0, t1 in zip(bounds[:-1], bounds[1:]):
        rects = []
        t = t0
        while t < t1:
            tr, tc = divmod(t, tpr)
            if tc == 0 and t1 - t >= tpr:
                nrow = (t1 - t) // tpr
                rects.append((tr * 8, nrow * 8, 0, C))
                t += nrow * tpr
            else:
                n = min(tpr - tc, t1 - t)
                rects.append((tr * 8, 8, tc * 128, n * 128))
                t += n
        pieces.append(rects)
    return pieces


def _stride_order(lst, s):
    return [lst[j] for off in range(s) for j in range(off, len(lst), s)]


def _merge(*ls):
    pos = []
    for a, l in enumerate(ls):
        for i, e in enumerate(l):
            pos.append(((i + 0.5) / len(l), a, e))
    pos.sort(key=lambda t: (t[0], t[1]))
    return [e for _, _, e in pos]


@jax.jit
def pallas_gated_mix__sliding_block_cached__glu_gated_swiglu__decode_kernel(
    A_x: jax.Array,
    A_k_cache: jax.Array,
    A_v_cache: jax.Array,
    A_wq: jax.Array,
    A_wo: jax.Array,
    B_x: jax.Array,
    B_w1: jax.Array,
    B_w3: jax.Array,
    B_w2: jax.Array,
    gate_w: jax.Array,
):
    del B_x
    B, Sq, D = A_x.shape
    _, H, SK, DH = A_k_cache.shape
    F = B_w1.shape[1]
    W = min(4096, max(256, SK // 4))
    assert B == 1 and Sq == 1 and A_wq.shape[1] == H * DH
    assert W == 2 * _COLS and DH % 8 == 0 and F == 128 * sum(_TAIL)
    scale = DH ** -0.5
    GS = DH // 8
    TOT = 4 * GS
    assert _LAG <= 3 * GS and H % 2 == 0

    kT = jnp.swapaxes(A_k_cache, 2, 3).reshape(H * DH, SK)
    vT = jnp.swapaxes(A_v_cache, 2, 3).reshape(H * DH, SK)

    def kernel(x_ref, k_ref, v_ref, wq_ref, wo_ref, w1_ref, w3_ref, w2_ref, gw_ref, o_ref,
               kvbuf, wq_b, wo_b, w1_b, w3_b, w2_b, x_b, gw_b, q_f, q_s, s_s, hh_s, sem):

        def kv_copy(h, j):
            st, r = j // GS, j % GS
            m, c = st // 2, st % 2
            src = k_ref if m == 0 else v_ref
            row = h * DH + r * 8
            if not isinstance(row, int):
                row = pl.multiple_of(row, 8)
            return pltpu.make_async_copy(
                src.at[pl.ds(row, 8), pl.ds(SK - W + c * _COLS, _COLS)],
                kvbuf.at[(h % 2) * 2 + m, pl.ds(r * 8, 8), pl.ds(c * _COLS, _COLS)],
                sem.at[st])

        def w_pieces(src, dst, **kw):
            R, C = src.shape
            return [[(src.at[pl.ds(r, nr), pl.ds(c, nc)], dst.at[pl.ds(r, nr), pl.ds(c, nc)])
                     for (r, nr, c, nc) in pc] for pc in _aligned_pieces(R, C, **kw)]

        p_wq = _stride_order(w_pieces(wq_ref, wq_b), _STRIDE)
        p_wo = _stride_order(w_pieces(wo_ref, wo_b), _STRIDE)
        p_w1 = _stride_order(w_pieces(w1_ref, w1_b), _STRIDE)
        p_w3 = _stride_order(w_pieces(w3_ref, w3_b), _STRIDE)
        third = len(p_wo) // 3
        groups = [
            [[(x_ref, x_b), (gw_ref, gw_b)]] + _merge(p_wq, p_wo[:third]),
            _merge(p_w1, p_w3, p_wo[third:2 * third]),
            p_wo[2 * third:],
        ]
        NPG = len(groups)
        stream = []
        for g, lst in enumerate(groups):
            stream += [("w", pc, g) for pc in lst]
        P = len(stream)
        for h in range(H):
            stream += [("kv", (h, j), NPG + 4 * h + j // GS) for j in range(TOT)]
        tail_groups = []
        r0 = 0
        for t, nk in enumerate(_TAIL):
            pcs = w_pieces(w2_ref, w2_b, r0=r0, r1=r0 + nk * 128)
            stream += [("w", pc, NPG + 4 * H + t) for pc in pcs]
            tail_groups.append((r0, nk * 128, len(stream)))
            r0 += nk * 128
        NTOT = len(stream)
        gend = {}
        for i, e in enumerate(stream):
            gend[e[2]] = i + 1

        def copies(i):
            kind, a, g = stream[i]
            if kind == "kv":
                return [kv_copy(*a)]
            return [pltpu.make_async_copy(s_, d_, sem.at[(g - NPG) % _NSEM]) for (s_, d_) in a]

        def prio(i):
            return 1 if stream[i][2] >= NPG + 4 * H + _TAIL_P1_FROM else i % 2

        st8 = {"started": 0, "waited": 0}

        def start_more():
            while st8["started"] < NTOT and st8["started"] - st8["waited"] < _LAG:
                i = st8["started"]
                prev = stream[i][2] - _NSEM
                if prev >= 0 and st8["waited"] < gend[prev]:
                    break
                for cp in copies(i):
                    cp.start(priority=prio(i))
                st8["started"] += 1

        def wait_until(n):
            while st8["waited"] < n:
                i = st8["waited"]
                assert i < st8["started"]
                for cp in copies(i):
                    cp.wait()
                st8["waited"] += 1
                start_more()

        def wait_with_tasks(n_end, tasks):
            n0 = st8["waited"]
            for i, task in enumerate(tasks):
                wait_until(n0 + (n_end - n0) * (i + 1) // (len(tasks) + 1))
                task()
            wait_until(n_end)

        start_more()

        wait_until(gend[0])
        x = x_b[0]
        xb = jnp.broadcast_to(x, (8, D))
        gw = gw_b[...].reshape(1, D).astype(_F32)
        gate = jax.nn.sigmoid(jnp.sum(x.astype(_F32) * gw, axis=-1, keepdims=True))

        def q_task(n0, n):
            def run():
                q_f[:, n0:n0 + n] = jnp.dot(xb, wq_b[:, n0:n0 + n],
                                            preferred_element_type=_F32).astype(_BF16)
            return run

        def q_split_heads():
            for h in range(H):
                q_s[h] = q_f[:, h * DH:(h + 1) * DH]

        def ffn_task(n0, n):
            def run():
                g_ = jnp.dot(xb, w1_b[:, n0:n0 + n], preferred_element_type=_F32)
                u_ = jnp.dot(xb, w3_b[:, n0:n0 + n], preferred_element_type=_F32)
                hh_s[:, n0:n0 + n] = (g_ * jax.nn.sigmoid(g_) * u_).astype(_BF16)
            return run

        wait_with_tasks(gend[1], [q_task(n0, 512) for n0 in range(0, H * DH, 512)] + [q_split_heads])
        wait_with_tasks(gend[2], [ffn_task(n0, 256) for n0 in range(0, F, 256)])

        par = P % 2

        def head(h, acc, static):
            def wait_group(st):
                if static:
                    wait_until(P + h * TOT + (st + 1) * GS)
                else:
                    for j in range(st * GS, (st + 1) * GS):
                        kv_copy(h, j).wait()
                        jn = j + _LAG
                        kv_copy(h + jn // TOT, jn % TOT).start(priority=(jn + par) % 2)

            kb = kvbuf.at[(h % 2) * 2]
            vb = kvbuf.at[(h % 2) * 2 + 1]

            def qk(c):
                n0 = c * _COLS
                s = jnp.dot(q_s[h], kb[:, n0:n0 + _COLS], preferred_element_type=_F32) * scale
                s_s[:, n0:n0 + _COLS] = s
                mm = s[:, 0:128]
                for u in range(1, _COLS // 128):
                    mm = jnp.maximum(mm, s[:, u * 128:(u + 1) * 128])
                return mm

            def pv(c, mx):
                n0 = c * _COLS
                e = jnp.exp(s_s[:, n0:n0 + _COLS] - mx)
                ll = e[:, 0:128]
                for u in range(1, _COLS // 128):
                    ll = ll + e[:, u * 128:(u + 1) * 128]
                o = lax.dot_general(e.astype(_BF16), vb[:, n0:n0 + _COLS], _NT,
                                    preferred_element_type=_F32)
                return ll, o

            wait_group(0)
            m0 = qk(0)
            wait_group(1)
            m1 = qk(1)
            mx = jnp.max(jnp.maximum(m0, m1), axis=-1, keepdims=True)
            wait_group(2)
            l0, o0 = pv(0, mx)
            wait_group(3)
            l1, o1 = pv(1, mx)
            l = jnp.sum(l0 + l1, axis=-1, keepdims=True)
            o = ((o0 + o1) / l).astype(_BF16)
            row = h * DH
            if not isinstance(row, int):
                row = pl.multiple_of(row, 64)
            return acc + jnp.dot(o, wo_b[pl.ds(row, DH), :], preferred_element_type=_F32)

        assert st8["waited"] == P and st8["started"] == P + _LAG
        acc = lax.fori_loop(0, H - 1, lambda h, a: head(h, a, False), jnp.zeros((8, D), _F32))
        st8["waited"] += (H - 1) * TOT
        st8["started"] += (H - 1) * TOT
        acc = head(H - 1, acc, True)

        ga = gate * acc[0:1]
        omg = 1.0 - gate
        b = None
        for (r0_, nr, i_end) in tail_groups:
            wait_until(i_end)
            pb = jnp.dot(hh_s[:, r0_:r0_ + nr], w2_b[r0_:r0_ + nr, :], preferred_element_type=_F32)
            b = pb if b is None else b + pb
        assert st8["waited"] == NTOT and st8["started"] == NTOT
        o_ref[0] = (ga + omg * b[0:1]).astype(o_ref.dtype)

    hbm = pl.BlockSpec(memory_space=pl.ANY)
    return pl.pallas_call(
        kernel,
        out_shape=jax.ShapeDtypeStruct((B, Sq, D), A_x.dtype),
        in_specs=[hbm] * 9,
        out_specs=pl.BlockSpec(memory_space=pltpu.VMEM),
        scratch_shapes=[
            pltpu.VMEM((4, DH, W), _BF16),
            pltpu.VMEM((D, H * DH), _BF16),
            pltpu.VMEM((H * DH, D), _BF16),
            pltpu.VMEM((D, F), _BF16),
            pltpu.VMEM((D, F), _BF16),
            pltpu.VMEM((F, D), _BF16),
            pltpu.VMEM((1, 1, D), _BF16),
            pltpu.VMEM((D,), _BF16),
            pltpu.VMEM((8, H * DH), _BF16),
            pltpu.VMEM((H, 8, DH), _BF16),
            pltpu.VMEM((8, W), _F32),
            pltpu.VMEM((8, F), _BF16),
            pltpu.SemaphoreType.DMA((_NSEM,)),
        ],
        compiler_params=pltpu.CompilerParams(vmem_limit_bytes=48 * 1024 * 1024),
    )(A_x, kT, vT, A_wq, A_wo, B_w1, B_w3, B_w2, gate_w)
```

```python
import jax
import jax.numpy as jnp
from jax import lax
import jax.experimental.pallas as pl
import jax.experimental.pallas.tpu as pltpu

_NT = (((1,), (1,)), ((), ()))
_F32 = jnp.float32
_BF16 = jnp.bfloat16

_LAG = 72
_NSEM = 4
_COLS = 2048
_STRIDE = 16
_TAIL = (6, 3, 2, 1)
_TAIL_P1_FROM = 2
_NPRE = 8
_SUB = 4


def _aligned_pieces(R, C, r0=0, r1=None, ntiles=16):
    r1 = R if r1 is None else r1
    tpr = C // 128
    ta, tb = (r0 // 8) * tpr, (r1 // 8) * tpr
    bounds = sorted(set([ta, tb] + [t for t in range(0, (R // 8) * tpr + 1, ntiles) if ta < t < tb]))
    pieces = []
    for t0, t1 in zip(bounds[:-1], bounds[1:]):
        rects = []
        t = t0
        while t < t1:
            tr, tc = divmod(t, tpr)
            if tc == 0 and t1 - t >= tpr:
                nrow = (t1 - t) // tpr
                rects.append((tr * 8, nrow * 8, 0, C))
                t += nrow * tpr
            else:
                n = min(tpr - tc, t1 - t)
                rects.append((tr * 8, 8, tc * 128, n * 128))
                t += n
        pieces.append(rects)
    return pieces


def _stride_order(lst, s):
    return [lst[j] for off in range(s) for j in range(off, len(lst), s)]


def _merge(*ls):
    pos = []
    for a, l in enumerate(ls):
        for i, e in enumerate(l):
            pos.append(((i + 0.5) / len(l), a, e))
    pos.sort(key=lambda t: (t[0], t[1]))
    return [e for _, _, e in pos]


@jax.jit
def pallas_gated_mix__sliding_block_cached__glu_gated_swiglu__decode_kernel(
    A_x: jax.Array,
    A_k_cache: jax.Array,
    A_v_cache: jax.Array,
    A_wq: jax.Array,
    A_wo: jax.Array,
    B_x: jax.Array,
    B_w1: jax.Array,
    B_w3: jax.Array,
    B_w2: jax.Array,
    gate_w: jax.Array,
):
    del B_x
    B, Sq, D = A_x.shape
    _, H, SK, DH = A_k_cache.shape
    F = B_w1.shape[1]
    W = min(4096, max(256, SK // 4))
    assert B == 1 and Sq == 1 and A_wq.shape[1] == H * DH
    assert W == 2 * _COLS and DH % 8 == 0 and F == 128 * sum(_TAIL)
    scale = DH ** -0.5
    GS = DH // 8
    TOT = 4 * GS
    assert _LAG <= 3 * GS and _LAG + _NPRE <= 4 * GS and _NPRE <= GS and H % 2 == 0
    assert _TAIL[-1] == 1 and len(_TAIL) <= _NSEM

    kT = jnp.swapaxes(A_k_cache, 2, 3).reshape(H * DH, SK)
    vT = jnp.swapaxes(A_v_cache, 2, 3).reshape(H * DH, SK)

    def kernel(x_ref, k_ref, v_ref, wq_ref, wo_ref, w1_ref, w3_ref, w2_ref, gw_ref, o_ref,
               kvbuf, wq_b, wo_b, w1_b, w3_b, w2_b, x_b, gw_b, q_f, q_s, s_s, hh_s, sem):

        def kv_copy(h, j):
            st, r = j // GS, j % GS
            m, c = st // 2, st % 2
            src = k_ref if m == 0 else v_ref
            row = h * DH + r * 8
            if not isinstance(row, int):
                row = pl.multiple_of(row, 8)
            return pltpu.make_async_copy(
                src.at[pl.ds(row, 8), pl.ds(SK - W + c * _COLS, _COLS)],
                kvbuf.at[(h % 2) * 2 + m, pl.ds(r * 8, 8), pl.ds(c * _COLS, _COLS)],
                sem.at[st])

        def w_pieces(src, dst, **kw):
            R, C = src.shape
            return [[(src.at[pl.ds(r, nr), pl.ds(c, nc)], dst.at[pl.ds(r, nr), pl.ds(c, nc)])
                     for (r, nr, c, nc) in pc] for pc in _aligned_pieces(R, C, **kw)]

        p_wq = _stride_order(w_pieces(wq_ref, wq_b), _STRIDE)
        p_wo = _stride_order(w_pieces(wo_ref, wo_b), _STRIDE)
        p_w1 = _stride_order(w_pieces(w1_ref, w1_b), _STRIDE)
        p_w3 = _stride_order(w_pieces(w3_ref, w3_b), _STRIDE)
        third = len(p_wo) // 3
        groups = [
            [[(x_ref, x_b), (gw_ref, gw_b)]] + _merge(p_wq, p_wo[:third]),
            _merge(p_w1, p_w3, p_wo[third:2 * third]),
            p_wo[2 * third:],
        ]
        NPG = len(groups)
        stream = []
        for g, lst in enumerate(groups):
            stream += [("w", pc, g) for pc in lst]
        P = len(stream)
        for h in range(H):
            stream += [("kv", (h, j), NPG + 4 * h + j // GS) for j in range(TOT)]
        tail_groups = []
        r0 = 0
        for t, nk in enumerate(_TAIL):
            pcs = w_pieces(w2_ref, w2_b, r0=r0, r1=r0 + nk * 128)
            stream += [("w", pc, NPG + 4 * H + t) for pc in pcs]
            tail_groups.append((r0, nk * 128, len(stream)))
            r0 += nk * 128
        NTOT = len(stream)
        gend = {}
        for i, e in enumerate(stream):
            gend[e[2]] = i + 1

        def copies(i):
            kind, a, g = stream[i]
            if kind == "kv":
                return [kv_copy(*a)]
            return [pltpu.make_async_copy(s_, d_, sem.at[(g - NPG) % _NSEM]) for (s_, d_) in a]

        def prio(i):
            return 1 if stream[i][2] >= NPG + 4 * H + _TAIL_P1_FROM else i % 2

        st8 = {"started": 0, "waited": 0}

        def start_more():
            while st8["started"] < NTOT and st8["started"] - st8["waited"] < _LAG:
                i = st8["started"]
                prev = stream[i][2] - _NSEM
                if prev >= 0 and st8["waited"] < gend[prev]:
                    break
                for cp in copies(i):
                    cp.start(priority=prio(i))
                st8["started"] += 1

        def wait_until(n):
            while st8["waited"] < n:
                i = st8["waited"]
                assert i < st8["started"]
                for cp in copies(i):
                    cp.wait()
                st8["waited"] += 1
                start_more()

        def wait_with_tasks(n_end, tasks):
            n0 = st8["waited"]
            for i, task in enumerate(tasks):
                wait_until(n0 + (n_end - n0) * (i + 1) // (len(tasks) + 1))
                task()
            wait_until(n_end)

        start_more()

        wait_until(gend[0])
        x = x_b[0]
        xb = jnp.broadcast_to(x, (8, D))
        gw = gw_b[...].reshape(1, D).astype(_F32)
        gate = jax.nn.sigmoid(jnp.sum(x.astype(_F32) * gw, axis=-1, keepdims=True))

        def q_task(n0, n):
            def run():
                q_f[:, n0:n0 + n] = jnp.dot(xb, wq_b[:, n0:n0 + n],
                                            preferred_element_type=_F32).astype(_BF16)
            return run

        def q_split_heads():
            for h in range(H):
                q_s[h] = q_f[:, h * DH:(h + 1) * DH]

        def ffn_task(n0, n):
            def run():
                g_ = jnp.dot(xb, w1_b[:, n0:n0 + n], preferred_element_type=_F32)
                u_ = jnp.dot(xb, w3_b[:, n0:n0 + n], preferred_element_type=_F32)
                hh_s[:, n0:n0 + n] = (g_ * jax.nn.sigmoid(g_) * u_).astype(_BF16)
            return run

        wait_with_tasks(gend[1], [q_task(n0, 512) for n0 in range(0, H * DH, 512)] + [q_split_heads])
        wait_with_tasks(gend[2], [ffn_task(n0, 256) for n0 in range(0, F, 256)])

        par = P % 2

        def kv_start(h, jn):
            kv_copy(h + jn // TOT, jn % TOT).start(priority=(jn + par) % 2)

        def head(h, acc, static):
            def wait_group(st):
                if static:
                    wait_until(P + h * TOT + (st + 1) * GS)
                    return
                for j in range(st * GS, (st + 1) * GS):
                    kv_copy(h, j).wait()
                    if j - st * GS >= _NPRE:
                        kv_start(h, j + _LAG)

            def early_starts(st_next, part):
                if static:
                    return
                for i in range(_NPRE * part // _SUB, _NPRE * (part + 1) // _SUB):
                    kv_start(h, st_next * GS + _LAG + i)

            kb = kvbuf.at[(h % 2) * 2]
            vb = kvbuf.at[(h % 2) * 2 + 1]
            cw = _COLS // _SUB

            def qk(c):
                mm = None
                for part in range(_SUB):
                    n0 = c * _COLS + part * cw
                    s = jnp.dot(q_s[h], kb[:, n0:n0 + cw], preferred_element_type=_F32) * scale
                    s_s[:, n0:n0 + cw] = s
                    for u in range(cw // 128):
                        t = s[:, u * 128:(u + 1) * 128]
                        mm = t if mm is None else jnp.maximum(mm, t)
                    early_starts(c + 1, part)
                return mm

            def pv(c, mx):
                ll = o = None
                for part in range(_SUB):
                    n0 = c * _COLS + part * cw
                    e = jnp.exp(s_s[:, n0:n0 + cw] - mx)
                    for u in range(cw // 128):
                        t = e[:, u * 128:(u + 1) * 128]
                        ll = t if ll is None else ll + t
                    o_ = lax.dot_general(e.astype(_BF16), vb[:, n0:n0 + cw], _NT,
                                         preferred_element_type=_F32)
                    o = o_ if o is None else o + o_
                    early_starts(c + 3, part)
                return ll, o

            wait_group(0)
            m0 = qk(0)
            wait_group(1)
            m1 = qk(1)
            mx = jnp.max(jnp.maximum(m0, m1), axis=-1, keepdims=True)
            wait_group(2)
            l0, o0 = pv(0, mx)
            wait_group(3)
            l1, o1 = pv(1, mx)
            l = jnp.sum(l0 + l1, axis=-1, keepdims=True)
            o = ((o0 + o1) / l).astype(_BF16)
            row = h * DH
            if not isinstance(row, int):
                row = pl.multiple_of(row, 64)
            return acc + jnp.dot(o, wo_b[pl.ds(row, DH), :], preferred_element_type=_F32)

        assert st8["waited"] == P and st8["started"] == P + _LAG
        for _ in range(_NPRE):
            for cp in copies(st8["started"]):
                cp.start(priority=prio(st8["started"]))
            st8["started"] += 1
        acc = lax.fori_loop(0, H - 1, lambda h, a: head(h, a, False), jnp.zeros((8, D), _F32))
        st8["waited"] += (H - 1) * TOT
        st8["started"] += (H - 1) * TOT
        acc = head(H - 1, acc, True)

        hrow = hh_s[0:1, F - 128:F].astype(_F32)
        hcol = jnp.transpose(jnp.broadcast_to(hrow, (128, 128)))
        b = None
        for (r0_, nr, i_end) in tail_groups[:-1]:
            wait_until(i_end)
            pb = jnp.dot(hh_s[:, r0_:r0_ + nr], w2_b[r0_:r0_ + nr, :], preferred_element_type=_F32)
            b = pb if b is None else b + pb
        omg = 1.0 - gate
        partial = gate * acc[0:1] + omg * b[0:1]
        wait_until(tail_groups[-1][2])
        assert st8["waited"] == NTOT and st8["started"] == NTOT
        w_last = w2_b[F - 128:F, :].astype(_F32)
        b_last = jnp.concatenate(
            [jnp.sum(w_last[:, n:n + 128] * hcol, axis=0, keepdims=True) for n in range(0, D, 128)],
            axis=1)
        o_ref[0] = (partial + omg * b_last).astype(o_ref.dtype)

    hbm = pl.BlockSpec(memory_space=pl.ANY)
    return pl.pallas_call(
        kernel,
        out_shape=jax.ShapeDtypeStruct((B, Sq, D), A_x.dtype),
        in_specs=[hbm] * 9,
        out_specs=pl.BlockSpec(memory_space=pltpu.VMEM),
        scratch_shapes=[
            pltpu.VMEM((4, DH, W), _BF16),
            pltpu.VMEM((D, H * DH), _BF16),
            pltpu.VMEM((H * DH, D), _BF16),
            pltpu.VMEM((D, F), _BF16),
            pltpu.VMEM((D, F), _BF16),
            pltpu.VMEM((F, D), _BF16),
            pltpu.VMEM((1, 1, D), _BF16),
            pltpu.VMEM((D,), _BF16),
            pltpu.VMEM((8, H * DH), _BF16),
            pltpu.VMEM((H, 8, DH), _BF16),
            pltpu.VMEM((8, W), _F32),
            pltpu.VMEM((8, F), _BF16),
            pltpu.SemaphoreType.DMA((_NSEM,)),
        ],
        compiler_params=pltpu.CompilerParams(vmem_limit_bytes=48 * 1024 * 1024),
    )(A_x, kT, vT, A_wq, A_wo, B_w1, B_w3, B_w2, gate_w)
```

```python
import jax
import jax.numpy as jnp
from jax import lax
import jax.experimental.pallas as pl
import jax.experimental.pallas.tpu as pltpu

_NT = (((1,), (1,)), ((), ()))
_F32 = jnp.float32
_BF16 = jnp.bfloat16

_LAG = 72
_NSEM = 4
_COLS = 2048
_STRIDE_BIG = 8
_STRIDE_SMALL = 20
_TAIL = (6, 3, 2, 1)
_TAIL_P1_FROM = 2
_NPRE = 8
_SUB = 4


def _aligned_pieces(R, C, r0=0, r1=None, ntiles=16):
    r1 = R if r1 is None else r1
    tpr = C // 128
    ta, tb = (r0 // 8) * tpr, (r1 // 8) * tpr
    bounds = sorted(set([ta, tb] + [t for t in range(0, (R // 8) * tpr + 1, ntiles) if ta < t < tb]))
    pieces = []
    for t0, t1 in zip(bounds[:-1], bounds[1:]):
        rects = []
        t = t0
        while t < t1:
            tr, tc = divmod(t, tpr)
            if tc == 0 and t1 - t >= tpr:
                nrow = (t1 - t) // tpr
                rects.append((tr * 8, nrow * 8, 0, C))
                t += nrow * tpr
            else:
                n = min(tpr - tc, t1 - t)
                rects.append((tr * 8, 8, tc * 128, n * 128))
                t += n
        pieces.append(rects)
    return pieces


def _stride_order(lst, s):
    return [lst[j] for off in range(s) for j in range(off, len(lst), s)]


def _merge(*ls):
    pos = []
    for a, l in enumerate(ls):
        for i, e in enumerate(l):
            pos.append(((i + 0.5) / len(l), a, e))
    pos.sort(key=lambda t: (t[0], t[1]))
    return [e for _, _, e in pos]


@jax.jit
def pallas_gated_mix__sliding_block_cached__glu_gated_swiglu__decode_kernel(
    A_x: jax.Array,
    A_k_cache: jax.Array,
    A_v_cache: jax.Array,
    A_wq: jax.Array,
    A_wo: jax.Array,
    B_x: jax.Array,
    B_w1: jax.Array,
    B_w3: jax.Array,
    B_w2: jax.Array,
    gate_w: jax.Array,
):
    del B_x
    B, Sq, D = A_x.shape
    _, H, SK, DH = A_k_cache.shape
    F = B_w1.shape[1]
    W = min(4096, max(256, SK // 4))
    assert B == 1 and Sq == 1 and A_wq.shape[1] == H * DH
    assert W == 2 * _COLS and DH % 8 == 0 and F == 128 * sum(_TAIL)
    scale = DH ** -0.5
    GS = DH // 8
    TOT = 4 * GS
    assert _LAG <= 3 * GS and _LAG + _NPRE <= 4 * GS and _NPRE <= GS and H % 2 == 0
    assert _TAIL[-1] == 1 and len(_TAIL) <= _NSEM

    kT = jnp.swapaxes(A_k_cache, 2, 3).reshape(H * DH, SK)
    vT = jnp.swapaxes(A_v_cache, 2, 3).reshape(H * DH, SK)

    def kernel(x_ref, k_ref, v_ref, wq_ref, wo_ref, w1_ref, w3_ref, w2_ref, gw_ref, o_ref,
               kvbuf, wq_b, wo_b, w1_b, w3_b, w2_b, x_b, gw_b, q_f, q_s, s_s, hh_s, sem):

        def kv_copy(h, j):
            st, r = j // GS, j % GS
            m, c = st // 2, st % 2
            src = k_ref if m == 0 else v_ref
            row = h * DH + r * 8
            if not isinstance(row, int):
                row = pl.multiple_of(row, 8)
            return pltpu.make_async_copy(
                src.at[pl.ds(row, 8), pl.ds(SK - W + c * _COLS, _COLS)],
                kvbuf.at[(h % 2) * 2 + m, pl.ds(r * 8, 8), pl.ds(c * _COLS, _COLS)],
                sem.at[st])

        def w_pieces(src, dst, **kw):
            R, C = src.shape
            return [[(src.at[pl.ds(r, nr), pl.ds(c, nc)], dst.at[pl.ds(r, nr), pl.ds(c, nc)])
                     for (r, nr, c, nc) in pc] for pc in _aligned_pieces(R, C, **kw)]

        p_wq = _stride_order(w_pieces(wq_ref, wq_b), _STRIDE_BIG)
        p_wo = _stride_order(w_pieces(wo_ref, wo_b), _STRIDE_BIG)
        p_w1 = _stride_order(w_pieces(w1_ref, w1_b), _STRIDE_SMALL)
        p_w3 = _stride_order(w_pieces(w3_ref, w3_b), _STRIDE_SMALL)
        groups = [
            [[(x_ref, x_b), (gw_ref, gw_b)]] + p_wq,
            _merge(p_w1, p_w3),
            p_wo,
        ]
        NPG = len(groups)
        stream = []
        for g, lst in enumerate(groups):
            stream += [("w", pc, g) for pc in lst]
        P = len(stream)
        for h in range(H):
            stream += [("kv", (h, j), NPG + 4 * h + j // GS) for j in range(TOT)]
        tail_groups = []
        r0 = 0
        for t, nk in enumerate(_TAIL):
            pcs = w_pieces(w2_ref, w2_b, r0=r0, r1=r0 + nk * 128)
            stream += [("w", pc, NPG + 4 * H + t) for pc in pcs]
            tail_groups.append((r0, nk * 128, len(stream)))
            r0 += nk * 128
        NTOT = len(stream)
        gend = {}
        for i, e in enumerate(stream):
            gend[e[2]] = i + 1

        def copies(i):
            kind, a, g = stream[i]
            if kind == "kv":
                return [kv_copy(*a)]
            return [pltpu.make_async_copy(s_, d_, sem.at[(g - NPG) % _NSEM]) for (s_, d_) in a]

        def prio(i):
            return 1 if stream[i][2] >= NPG + 4 * H + _TAIL_P1_FROM else i % 2

        st8 = {"started": 0, "waited": 0}

        def start_more():
            while st8["started"] < NTOT and st8["started"] - st8["waited"] < _LAG:
                i = st8["started"]
                prev = stream[i][2] - _NSEM
                if prev >= 0 and st8["waited"] < gend[prev]:
                    break
                for cp in copies(i):
                    cp.start(priority=prio(i))
                st8["started"] += 1

        def wait_until(n):
            while st8["waited"] < n:
                i = st8["waited"]
                assert i < st8["started"]
                for cp in copies(i):
                    cp.wait()
                st8["waited"] += 1
                start_more()

        def wait_with_tasks(n_end, tasks):
            n0 = st8["waited"]
            for i, task in enumerate(tasks):
                wait_until(n0 + (n_end - n0) * (i + 1) // (len(tasks) + 1))
                task()
            wait_until(n_end)

        start_more()

        wait_until(gend[0])
        x = x_b[0]
        xb = jnp.broadcast_to(x, (8, D))
        gw = gw_b[...].reshape(1, D).astype(_F32)
        gate = jax.nn.sigmoid(jnp.sum(x.astype(_F32) * gw, axis=-1, keepdims=True))

        def q_task(n0, n):
            def run():
                q_f[:, n0:n0 + n] = jnp.dot(xb, wq_b[:, n0:n0 + n],
                                            preferred_element_type=_F32).astype(_BF16)
            return run

        def q_split_heads():
            for h in range(H):
                q_s[h] = q_f[:, h * DH:(h + 1) * DH]

        def ffn_task(n0, n):
            def run():
                g_ = jnp.dot(xb, w1_b[:, n0:n0 + n], preferred_element_type=_F32)
                u_ = jnp.dot(xb, w3_b[:, n0:n0 + n], preferred_element_type=_F32)
                hh_s[:, n0:n0 + n] = (g_ * jax.nn.sigmoid(g_) * u_).astype(_BF16)
            return run

        wait_with_tasks(gend[1], [q_task(n0, 512) for n0 in range(0, H * DH, 512)] + [q_split_heads])
        wait_with_tasks(gend[2], [ffn_task(n0, 256) for n0 in range(0, F, 256)])

        par = P % 2

        def kv_start(h, jn):
            kv_copy(h + jn // TOT, jn % TOT).start(priority=(jn + par) % 2)

        def head(h, acc, static):
            def wait_group(st):
                if static:
                    wait_until(P + h * TOT + (st + 1) * GS)
                    return
                for j in range(st * GS, (st + 1) * GS):
                    kv_copy(h, j).wait()
                    if j - st * GS >= _NPRE:
                        kv_start(h, j + _LAG)

            def early_starts(st_next, part):
                if static:
                    return
                for i in range(_NPRE * part // _SUB, _NPRE * (part + 1) // _SUB):
                    kv_start(h, st_next * GS + _LAG + i)

            kb = kvbuf.at[(h % 2) * 2]
            vb = kvbuf.at[(h % 2) * 2 + 1]
            cw = _COLS // _SUB

            def qk(c):
                mm = None
                for part in range(_SUB):
                    n0 = c * _COLS + part * cw
                    s = jnp.dot(q_s[h], kb[:, n0:n0 + cw], preferred_element_type=_F32) * scale
                    s_s[:, n0:n0 + cw] = s
                    for u in range(cw // 128):
                        t = s[:, u * 128:(u + 1) * 128]
                        mm = t if mm is None else jnp.maximum(mm, t)
                    early_starts(c + 1, part)
                return mm

            def pv(c, mx):
                ll = o = None
                for part in range(_SUB):
                    n0 = c * _COLS + part * cw
                    e = jnp.exp(s_s[:, n0:n0 + cw] - mx)
                    for u in range(cw // 128):
                        t = e[:, u * 128:(u + 1) * 128]
                        ll = t if ll is None else ll + t
                    o_ = lax.dot_general(e.astype(_BF16), vb[:, n0:n0 + cw], _NT,
                                         preferred_element_type=_F32)
                    o = o_ if o is None else o + o_
                    early_starts(c + 3, part)
                return ll, o

            wait_group(0)
            m0 = qk(0)
            wait_group(1)
            m1 = qk(1)
            mx = jnp.max(jnp.maximum(m0, m1), axis=-1, keepdims=True)
            wait_group(2)
            l0, o0 = pv(0, mx)
            wait_group(3)
            l1, o1 = pv(1, mx)
            l = jnp.sum(l0 + l1, axis=-1, keepdims=True)
            o = ((o0 + o1) / l).astype(_BF16)
            row = h * DH
            if not isinstance(row, int):
                row = pl.multiple_of(row, 64)
            return acc + jnp.dot(o, wo_b[pl.ds(row, DH), :], preferred_element_type=_F32)

        assert st8["waited"] == P and st8["started"] == P + _LAG
        for _ in range(_NPRE):
            for cp in copies(st8["started"]):
                cp.start(priority=prio(st8["started"]))
            st8["started"] += 1
        acc = lax.fori_loop(0, H - 1, lambda h, a: head(h, a, False), jnp.zeros((8, D), _F32))
        st8["waited"] += (H - 1) * TOT
        st8["started"] += (H - 1) * TOT
        acc = head(H - 1, acc, True)

        hrow = hh_s[0:1, F - 128:F].astype(_F32)
        hcol = jnp.transpose(jnp.broadcast_to(hrow, (128, 128)))
        b = None
        for (r0_, nr, i_end) in tail_groups[:-1]:
            wait_until(i_end)
            pb = jnp.dot(hh_s[:, r0_:r0_ + nr], w2_b[r0_:r0_ + nr, :], preferred_element_type=_F32)
            b = pb if b is None else b + pb
        omg = 1.0 - gate
        partial = gate * acc[0:1] + omg * b[0:1]
        wait_until(tail_groups[-1][2])
        assert st8["waited"] == NTOT and st8["started"] == NTOT
        w_last = w2_b[F - 128:F, :].astype(_F32)
        b_last = jnp.concatenate(
            [jnp.sum(w_last[:, n:n + 128] * hcol, axis=0, keepdims=True) for n in range(0, D, 128)],
            axis=1)
        o_ref[0] = (partial + omg * b_last).astype(o_ref.dtype)

    hbm = pl.BlockSpec(memory_space=pl.ANY)
    return pl.pallas_call(
        kernel,
        out_shape=jax.ShapeDtypeStruct((B, Sq, D), A_x.dtype),
        in_specs=[hbm] * 9,
        out_specs=pl.BlockSpec(memory_space=pltpu.VMEM),
        scratch_shapes=[
            pltpu.VMEM((4, DH, W), _BF16),
            pltpu.VMEM((D, H * DH), _BF16),
            pltpu.VMEM((H * DH, D), _BF16),
            pltpu.VMEM((D, F), _BF16),
            pltpu.VMEM((D, F), _BF16),
            pltpu.VMEM((F, D), _BF16),
            pltpu.VMEM((1, 1, D), _BF16),
            pltpu.VMEM((D,), _BF16),
            pltpu.VMEM((8, H * DH), _BF16),
            pltpu.VMEM((H, 8, DH), _BF16),
            pltpu.VMEM((8, W), _F32),
            pltpu.VMEM((8, F), _BF16),
            pltpu.SemaphoreType.DMA((_NSEM,)),
        ],
        compiler_params=pltpu.CompilerParams(vmem_limit_bytes=48 * 1024 * 1024),
    )(A_x, kT, vT, A_wq, A_wo, B_w1, B_w3, B_w2, gate_w)
```
